```python
import os as _os
_os.environ.setdefault("JAX_PLATFORMS", "cpu")
import jax
import jax.numpy as jnp

def _softmax(x, axis=-1):
    return jax.nn.softmax(x, axis=axis)
def _gelu(x):
    return jax.nn.gelu(x, approximate=True)
def _silu(x):
    return jax.nn.silu(x)
def _sigmoid(x):
    return jax.nn.sigmoid(x)
def _layernorm(x, axis=-1, eps=1e-5):
    m = jnp.mean(x, axis=axis, keepdims=True)
    v = jnp.var(x, axis=axis, keepdims=True)
    return (x - m) / jnp.sqrt(v + eps)
def _scatter_add(tgt, idx, src, axis=0):
    return tgt.at[idx].add(src)
def _segment_sum(src, seg, n):
    return jax.ops.segment_sum(src, seg, n)
class _Rng:
    def __init__(self, key):
        self._k = key
    def _next(self):
        self._k, sub = jax.random.split(self._k)
        return sub
    def normal(self, shape):
        return jax.random.normal(self._next(), shape, dtype=jnp.bfloat16)
    def randint(self, lo, hi, shape):
        return jax.random.randint(self._next(), shape, lo, hi, dtype=jnp.int32)
    def uniform(self, shape, lo=0.0, hi=1.0):
        return jax.random.uniform(self._next(), shape, jnp.bfloat16, lo, hi)
    def permutation(self, n):
        return jax.random.permutation(self._next(), n)


kernel_name = 'standalone__fft_conv__vision'

def setup_inputs():
    _rng = _Rng(jax.random.key(int.from_bytes(__import__("os").urandom(4), "little")))
    _w = (lambda a: (lambda t: t.astype(jnp.bfloat16) if jnp.issubdtype(t.dtype, jnp.floating) else t)(jnp.asarray(a)))
    H = W = 224
    C = 96
    K = 3
    return {
        "x": _w((lambda *s: _rng.normal(s) * 0.05)(1, H, W, C)),
        "w": _w((lambda *s: _rng.normal(s) * 0.05)(K, K, C, C)),
    }

def reference(x, w):
    B, H, W, C = x.shape
    K = w.shape[0]
    wp = jnp.pad(w, ((0, H - K), (0, W - K), (0, 0), (0, 0)))
    Xf = (lambda x, axes=(-2,-1): jnp.fft.rfft2(x.astype(jnp.float32), axes=axes))(x, axes=(1, 2))
    Wf = (lambda x, axes=(-2,-1): jnp.fft.rfft2(x.astype(jnp.float32), axes=axes))(wp, axes=(0, 1))
    Yf = jnp.einsum('bhwi,hwio->bhwo', Xf, Wf)
    y = (lambda x, s, axes=(-2,-1): jnp.fft.irfft2(x, s=s, axes=axes).astype(jnp.bfloat16))(Yf, (H, W), axes=(1, 2))
    return y
```

```python
import functools
import numpy as np
import jax, jax.numpy as jnp
from jax.experimental import pallas as pl
from jax.experimental.pallas import tpu as pltpu

H = W = 224
C = 96
P_, Q_ = 1.5, 2.0 / 3.0
S_ = P_ * P_ + Q_ * Q_

def gcoefs():
    p, q = P_, Q_
    BT = np.array([
        [1, 0, -S_, 0, 1, 0],
        [0, -q, -q*q, p, 1, 0],
        [0, q, -q*q, -p, 1, 0],
        [0, -p, -p*p, q, 1, 0],
        [0, p, -p*p, -q, 1, 0],
        [0, 1, 0, -S_, 0, 1]], dtype=np.float64)
    pts = [0, p, -p, q, -q]
    AT = np.zeros((4, 6)); G = np.zeros((6, 3))
    for j, a in enumerate(pts):
        AT[:, j] = [a ** i for i in range(4)]
        nrm = np.prod([a - b for k, b in enumerate(pts) if k != j])
        G[j] = [a ** i / nrm for i in range(3)]
    AT[3, 5] = 1; G[5, 2] = 1
    for i in range(4):
        for k in range(3):
            v = (AT[i] * G[:, k]) @ BT
            e = np.zeros(6); e[i + k] = 1
            assert np.allclose(v, e), (i, k, v)
    return G
G_ = gcoefs()

def build(Q=4, wstart=0):
    NIT = (H // 4) // Q
    RB = 4 * Q
    def kern(x_hbm, w_hbm, o_hbm, xbuf, obuf, wbuf, u_ref, ua_ref, ur_ref, sem_w, sem_h, sem_in, sem_out):
        def in_copy(i):
            n = RB if i < NIT - 1 else RB - 2
            return pltpu.make_async_copy(x_hbm.at[pl.ds(i * RB, n)], xbuf.at[pl.ds(i * RB, n)], sem_in.at[i])
        def out_copy(i):
            return pltpu.make_async_copy(obuf.at[pl.ds(i * RB, RB)], o_hbm.at[pl.ds(i * RB, RB)], sem_out.at[i])
        wc = pltpu.make_async_copy(w_hbm, wbuf, sem_w)
        hc = pltpu.make_async_copy(x_hbm.at[pl.ds(H - 2, 2)], xbuf.at[pl.ds(H - 2, 2)], sem_h)
        wc.start(); hc.start()
        for i in range(NIT):
            in_copy(i).start(priority=1)
        wc.wait()
        eye = (jax.lax.broadcasted_iota(jnp.int32, (C, C), 0) == jax.lax.broadcasted_iota(jnp.int32, (C, C), 1)).astype(jnp.bfloat16)
        g = [jax.lax.dot_general(eye, wbuf[a * 3 * C:(a + 1) * 3 * C, :], (((1,), (1,)), ((), ())), preferred_element_type=jnp.float32) for a in range(3)]
        f = [g[2], g[1], g[0]]
        for j in range(1, 5):
            u = G_[j, 0] * f[0] + G_[j, 1] * f[1] + G_[j, 2] * f[2]
            u_ref[j - 1] = u[:, :256].astype(jnp.bfloat16)
        z = jnp.zeros((C, 32), jnp.float32)
        fr = [t[:, 256:] for t in f]
        r0 = jnp.concatenate(fr + [z], axis=1)
        r1 = jnp.concatenate([z] + fr, axis=1)
        ua_ref[0] = jnp.concatenate([f[0][:, :256], r0], axis=1).astype(jnp.bfloat16)
        ua_ref[1] = jnp.concatenate([f[2][:, :256], r1], axis=1).astype(jnp.bfloat16)
        ur_ref[0:C] = r0.astype(jnp.bfloat16)
        ur_ref[C:2 * C] = r1.astype(jnp.bfloat16)
        hc.wait()

        def load_row(h):
            t0 = pltpu.bitcast(xbuf[h, :, 0:128], jnp.uint32)
            t1 = pltpu.bitcast(xbuf[h, :, 128:224], jnp.uint32)
            return pltpu.bitcast(jnp.concatenate([t0, t1, t1[:, 64:]], axis=1), jnp.bfloat16)

        def shift(v, b):
            return pltpu.bitcast(pltpu.roll(pltpu.bitcast(v, jnp.uint32), b, axis=1), jnp.bfloat16)

        def stack(v, extra=()):
            v = v.astype(jnp.bfloat16)
            return jnp.concatenate([v, shift(v, 1), shift(v[:64], 2)] + list(extra), axis=0)

        dot = lambda a, b: jnp.dot(a, b, preferred_element_type=jnp.float32)

        def body(i, carry):
            @pl.when(i < NIT - 1)
            def _():
                pltpu.make_async_copy(x_hbm.at[pl.ds(0, RB)], xbuf.at[pl.ds(0, RB)], sem_in.at[i]).wait()
            @pl.when(i == NIT - 1)
            def _():
                in_copy(NIT - 1).wait()
            base = i * RB
            hm = jnp.where(i == 0, H - 2, base - 2)
            rows = {-2: load_row(hm), -1: load_row(hm + 1)}
            rems = {k: shift(rows[k][64:], 2) for k in rows}
            for t in range(Q):
                for k in range(4):
                    rows[4 * t + k] = load_row(base + 4 * t + k)
                    rems[4 * t + k] = shift(rows[4 * t + k][64:], 2)
                d = [rows[4 * t - 2 + k].astype(jnp.float32) for k in range(6)]
                r = [rems[4 * t - 2 + k] for k in range(6)]
                p, q = P_, Q_
                a2 = (p * p) * d[2]
                eq = d[4] - (q * q) * d[2]
                ep = d[4] - a2
                oq = p * d[3] - q * d[1]
                op = q * d[3] - p * d[1]
                v0 = d[0] + eq - a2
                v5 = (d[1] + d[5]) - S_ * d[3]
                m0 = dot(ua_ref[0], stack(v0, r[0:4]))
                m1 = dot(u_ref[0], stack(eq + oq))
                m2 = dot(u_ref[1], stack(eq - oq))
                m3 = dot(u_ref[2], stack(ep + op))
                m4 = dot(u_ref[3], stack(ep - op))
                m5 = dot(ua_ref[1], stack(v5, r[2:6]))
                rr = dot(ur_ref[...], jnp.concatenate(r[1:5], axis=0))
                s1, d1, s2, d2 = m1 + m2, m1 - m2, m3 + m4, m3 - m4
                y0 = m0 + s1 + s2
                y1 = p * d1 + q * d2 + rr[:C]
                y2 = (p * p) * s1 + (q * q) * s2 + rr[C:]
                y3 = (p ** 3) * d1 + (q ** 3) * d2 + m5
                for k, y in enumerate((y0, y1, y2, y3)):
                    obuf[base + 4 * t + k] = y[:, :W].astype(jnp.bfloat16)
            pltpu.make_async_copy(obuf.at[pl.ds(base, RB)], o_hbm.at[pl.ds(base, RB)], sem_out.at[i]).start()
            return carry
        jax.lax.fori_loop(0, NIT, body, 0)
        for i in range(NIT):
            out_copy(i).wait()

    @jax.jit
    def f(x, w):
        xt = jnp.transpose(x[0], (0, 2, 1))
        w2 = w.reshape(9 * C, C)
        yt = pl.pallas_call(
            kern,
            in_specs=[pl.BlockSpec(memory_space=pl.ANY), pl.BlockSpec(memory_space=pl.ANY)],
            out_specs=pl.BlockSpec(memory_space=pl.ANY),
            out_shape=jax.ShapeDtypeStruct((H, C, W), jnp.bfloat16),
            scratch_shapes=[
                pltpu.VMEM((H, C, W), jnp.bfloat16), pltpu.VMEM((H, C, W), jnp.bfloat16),
                pltpu.VMEM((9 * C, C), jnp.bfloat16),
                pltpu.VMEM((4, C, 256), jnp.bfloat16), pltpu.VMEM((2, C, 384), jnp.bfloat16), pltpu.VMEM((2 * C, 128), jnp.bfloat16),
                pltpu.SemaphoreType.DMA(()), pltpu.SemaphoreType.DMA(()),
                pltpu.SemaphoreType.DMA((NIT,)), pltpu.SemaphoreType.DMA((NIT,))],
            compiler_params=pltpu.CompilerParams(vmem_limit_bytes=64 * 1024 * 1024),
        )(xt, w2)
        return jnp.transpose(yt, (0, 2, 1))[None]
    return f


_impl = build(4)


@jax.jit
def pallas_standalone__fft_conv__vision_kernel(x: jax.Array, w: jax.Array):
    return _impl(x, w)
```

```python
import functools
import numpy as np
import jax, jax.numpy as jnp
from jax.experimental import pallas as pl
from jax.experimental.pallas import tpu as pltpu

H = W = 224
C = 96
NQ = H // 4
bf16, f32, u32 = jnp.bfloat16, jnp.float32, jnp.uint32

P_, Q_ = 1.5, 2.0 / 3.0
S_ = P_ * P_ + Q_ * Q_

def gcoefs():
    p, q = P_, Q_
    BT = np.array([
        [1, 0, -S_, 0, 1, 0],
        [0, -q, -q*q, p, 1, 0],
        [0, q, -q*q, -p, 1, 0],
        [0, -p, -p*p, q, 1, 0],
        [0, p, -p*p, -q, 1, 0],
        [0, 1, 0, -S_, 0, 1]], dtype=np.float64)
    pts = [0, p, -p, q, -q]
    AT = np.zeros((4, 6)); G = np.zeros((6, 3))
    for j, a in enumerate(pts):
        AT[:, j] = [a ** i for i in range(4)]
        nrm = np.prod([a - b for k, b in enumerate(pts) if k != j])
        G[j] = [a ** i / nrm for i in range(3)]
    AT[3, 5] = 1; G[5, 2] = 1
    for i in range(4):
        for k in range(3):
            v = (AT[i] * G[:, k]) @ BT
            e = np.zeros(6); e[i + k] = 1
            assert np.allclose(v, e), (i, k, v)
    return G
G_ = gcoefs()

def build(peel=(1, 2, 3), Q=5, qflush=24, PE=True, oprio=1, wfirst=True):
    NP = sum(peel)
    NIT = (NQ - NP) // Q
    assert NP + NIT * Q == NQ
    P = len(peel)
    RB = 4 * Q
    QM = max(max(peel), Q)
    sizes = list(peel) + [Q] * NIT
    starts = [sum(sizes[:b]) for b in range(len(sizes) + 1)]
    NB = len(sizes)
    assert qflush > NP
    i0, t0 = divmod(qflush - 1 - NP, Q)
    def kern(x_hbm, w_hbm, o_hbm, xbuf, obuf, wbuf, u_ref, ua_ref, ur_ref, v0_ref, v1_ref, r0_ref, r1_ref,
             sem_w, sem_h, sem_in, sem_out):
        v_refs = (v0_ref, v1_ref); r_refs = (r0_ref, r1_ref)
        def in_copy(b):
            lo = 4 * starts[b]
            n = min(4 * starts[b + 1], H - 2) - lo
            return pltpu.make_async_copy(x_hbm.at[pl.ds(lo, n)], xbuf.at[pl.ds(lo, n)], sem_in.at[b])
        wc = pltpu.make_async_copy(w_hbm, wbuf, sem_w)
        hc = pltpu.make_async_copy(x_hbm.at[pl.ds(H - 2, 2)], xbuf.at[pl.ds(H - 2, 2)], sem_h)
        wc.start(); hc.start(priority=1)
        for b in range(NB):
            in_copy(b).start(priority=1)
        eye = (jax.lax.broadcasted_iota(jnp.int32, (C, C), 0) == jax.lax.broadcasted_iota(jnp.int32, (C, C), 1)).astype(bf16)
        def wrows(a):
            wa = wbuf[a * 3 * C:(a + 1) * 3 * C, :]
            if not PE:
                return wa
            wf = wa.astype(f32)
            pieces = [pltpu.pack_elementwise([wf[16 * g:16 * g + 8], wf[16 * g + 8:16 * g + 16]], packed_dtype=bf16) for g in range(16)]
            return jnp.concatenate([pltpu.bitcast(jnp.concatenate(pieces, axis=0), bf16), wa[256:]], axis=0)
        def prep_w():
            g = [jax.lax.dot_general(eye, wrows(a), (((1,), (1,)), ((), ())), preferred_element_type=f32) for a in range(3)]
            f = [g[2], g[1], g[0]]
            tou = lambda t: pltpu.bitcast(t.astype(bf16), u32)
            for j in range(1, 5):
                u = G_[j, 0] * f[0] + G_[j, 1] * f[1] + G_[j, 2] * f[2]
                u_ref[j - 1] = tou(u[:, :256])
            z = jnp.zeros((C, 32), f32)
            fr = [t[:, 256:] for t in f]
            r0 = jnp.concatenate(fr + [z], axis=1)
            r1 = jnp.concatenate([z] + fr, axis=1)
            ua_ref[0] = tou(jnp.concatenate([f[0][:, :256], r0], axis=1))
            ua_ref[1] = tou(jnp.concatenate([f[2][:, :256], r1], axis=1))
            ur_ref[0:C // 2] = tou(r0)
            ur_ref[C // 2:C] = tou(r1)

        p, q = P_, Q_
        def xform(d):
            a2 = (p * p) * d[2]
            eq = d[4] - (q * q) * d[2]
            ep = d[4] - a2
            oq = p * d[3] - q * d[1]
            op = q * d[3] - p * d[1]
            return [d[0] + eq - a2, eq + oq, eq - oq, ep + op, ep - op, (d[1] + d[5]) - S_ * d[3]]
        sh = lambda u, b: jnp.concatenate([u[:, W - b:], u[:, :W - b]], axis=1)

        def stage_a(hs, slot, t):
            v_ref, r_ref = v_refs[slot], r_refs[slot]
            def rem(k):
                r_ref[16 * (4 * t + k):16 * (4 * t + k) + 16, :W] = sh(pltpu.bitcast(xbuf[hs[k], 64:96, :], u32), 2)
            ks = list(range(6)) if t == 0 else list(range(2, 6))
            pend = None
            for g in (0, 1, 2, 3, 4, 5):
                c0_ = 16 * g
                if PE:
                    halves = []
                    for hf in range(2):
                        d = [xbuf[h, c0_ + 8 * hf:c0_ + 8 * hf + 8, :].astype(f32) for h in hs]
                        halves.append(xform(d))
                    us = [pltpu.pack_elementwise([halves[0][j], halves[1][j]], packed_dtype=bf16) for j in range(6)]
                else:
                    d = [xbuf[h, c0_:c0_ + 16, :].astype(f32) for h in hs]
                    us = [pltpu.bitcast(v.astype(bf16), u32) for v in xform(d)]
                for j in range(6):
                    v_ref[t * 6 + j, 8 * g:8 * g + 8, :W] = us[j]
                if g < 4:
                    es = [jnp.concatenate([u, u[:, 192:]], axis=1) for u in us]
                else:
                    for j in range(6):
                        v_ref[t * 6 + j, 48 + 8 * g:48 + 8 * g + 8, :W] = sh(us[j], 1)
                if g == 0:
                    for k in ks: rem(k)
                if pend is not None:
                    pg, pes = pend
                    for j in range(6):
                        v_ref[t * 6 + j, 48 + 8 * pg:48 + 8 * pg + 8, :] = pltpu.roll(pes[j], 1, axis=1)
                        v_ref[t * 6 + j, 96 + 8 * pg:96 + 8 * pg + 8, :] = pltpu.roll(pes[j], 2, axis=1)
                pend = (g, es) if g < 4 else None

        tob = lambda t: pltpu.bitcast(t, bf16)
        dot = lambda a, b: jnp.dot(tob(a), tob(b), preferred_element_type=f32)
        def stage_b(h0, slot, t):
            v_ref, r_ref = v_refs[slot], r_refs[slot]
            rb = 64 * t
            for (l0, l1) in [(0, 128), (128, W)]:
                m = {j: dot(u_ref[j - 1], v_ref[t * 6 + j, :, l0:l1]) for j in range(1, 5)}
                s1, d1, s2, d2 = m[1] + m[2], m[1] - m[2], m[3] + m[4], m[3] - m[4]
                m0 = dot(ua_ref[0], jnp.concatenate([v_ref[t * 6, :, l0:l1], r_ref[rb:rb + 64, l0:l1]], axis=0))
                obuf[h0, :, l0:l1] = ((s1 + s2) + m0).astype(bf16)
                rr = dot(ur_ref[...], r_ref[rb + 16:rb + 80, l0:l1])
                obuf[h0 + 1, :, l0:l1] = ((p * d1 + q * d2) + rr[:C]).astype(bf16)
                obuf[h0 + 2, :, l0:l1] = (((p * p) * s1 + (q * q) * s2) + rr[C:]).astype(bf16)
                m5 = dot(ua_ref[1], jnp.concatenate([v_ref[t * 6 + 5, :, l0:l1], r_ref[rb + 32:rb + 96, l0:l1]], axis=0))
                obuf[h0 + 3, :, l0:l1] = (((p ** 3) * d1 + (q ** 3) * d2) + m5).astype(bf16)

        def out_start(lo, n):
            pltpu.make_async_copy(obuf.at[pl.ds(lo, n)], o_hbm.at[pl.ds(lo, n)], sem_out).start(priority=oprio)

        if wfirst:
            wc.wait(); prep_w()
            hc.wait(); in_copy(0).wait()
        else:
            wc.wait(); hc.wait(); in_copy(0).wait()
        for t in range(sizes[0]):
            stage_a([(4 * t - 2 + k) % H for k in range(6)], 0, t)
        if not wfirst:
            prep_w()
        for b in range(P):
            in_copy(b + 1).wait()
            for t in range(max(sizes[b], sizes[b + 1])):
                if t < sizes[b]:
                    stage_b(4 * (starts[b] + t), b % 2, t)
                if t < sizes[b + 1]:
                    stage_a([4 * (starts[b + 1] + t) - 2 + k for k in range(6)], (b + 1) % 2, t)

        def body(i, carry):
            @pl.when(i < NIT - 2)
            def _():
                lo = 4 * NP + (i + 1) * RB
                pltpu.make_async_copy(x_hbm.at[pl.ds(lo, RB)], xbuf.at[pl.ds(lo, RB)], sem_in.at[P + 1 + i]).wait()
            @pl.when(i == NIT - 2)
            def _():
                in_copy(NB - 1).wait()
            base = 4 * NP + i * RB
            nbase = jnp.minimum(base + RB, H - RB)
            def half(s):
                for t in range(Q):
                    stage_b(base + 4 * t, s, t)
                    if t == t0 and (P + i0) % 2 == s:
                        pl.when(i == i0)(lambda: out_start(0, 4 * qflush))
                    pl.when(i > i0 if t <= t0 else i >= i0)(lambda: out_start(base + 4 * t, 4))
                    stage_a([nbase + 4 * t - 2 + k for k in range(6)], 1 - s, t)
            pl.when((i + P) % 2 == 0)(lambda: half(0))
            pl.when((i + P) % 2 == 1)(lambda: half(1))
            return carry
        jax.lax.fori_loop(0, NIT, body, 0)
        pltpu.make_async_copy(obuf, o_hbm, sem_out).wait()

    @jax.jit
    def f(x, w):
        xt = jnp.transpose(x[0], (0, 2, 1))
        w2 = w.reshape(9 * C, C)
        yt = pl.pallas_call(
            kern,
            in_specs=[pl.BlockSpec(memory_space=pl.ANY), pl.BlockSpec(memory_space=pl.ANY)],
            out_specs=pl.BlockSpec(memory_space=pl.ANY),
            out_shape=jax.ShapeDtypeStruct((H, C, W), bf16),
            scratch_shapes=[
                pltpu.VMEM((H, C, W), bf16), pltpu.VMEM((H, C, W), bf16),
                pltpu.VMEM((9 * C, C), bf16),
                pltpu.VMEM((4, C // 2, 256), u32), pltpu.VMEM((2, C // 2, 384), u32), pltpu.VMEM((C, 128), u32),
                pltpu.VMEM((QM * 6, 128, 256), u32), pltpu.VMEM((QM * 6, 128, 256), u32),
                pltpu.VMEM((64 * QM + 32, 256), u32), pltpu.VMEM((64 * QM + 32, 256), u32),
                pltpu.SemaphoreType.DMA(()), pltpu.SemaphoreType.DMA(()),
                pltpu.SemaphoreType.DMA((NB,)), pltpu.SemaphoreType.DMA(())],
            compiler_params=pltpu.CompilerParams(vmem_limit_bytes=100 * 1024 * 1024, disable_bounds_checks=True),
        )(xt, w2)
        return jnp.transpose(yt, (0, 2, 1))[None]
    return f


_impl = build((1, 2, 3, 4, 6), 8, 22)


@jax.jit
def pallas_standalone__fft_conv__vision_kernel(x: jax.Array, w: jax.Array):
    return _impl(x, w)
```

```python
import functools

import numpy as np
import jax
import jax.numpy as jnp
import jax.experimental.pallas as pl
import jax.experimental.pallas.tpu as pltpu

H = W = 224
C = 96
NQ = H // 4
WP = 256
bf16, f32, u32 = jnp.bfloat16, jnp.float32, jnp.uint32

P_ = 1.75
Q_ = 1.0 / P_
S_ = P_ * P_ + Q_ * Q_
Z, I, PP, PM, QP, QM, RP, RM = range(8)


def _xf_s(d):
    p, q = P_, Q_
    a2 = (p * p) * d[2]
    eq = d[4] - (q * q) * d[2]
    ep = d[4] - a2
    oq = p * d[3] - q * d[1]
    op = q * d[3] - p * d[1]
    return {Z: d[0] + eq - a2, PP: eq + oq, PM: eq - oq, QP: ep + op, QM: ep - op,
            I: (d[1] + d[5]) - S_ * d[3]}


def _xf_a1(d, a, dp, dm):
    e1 = d[4] - (a * a) * d[2]
    o1 = d[3] - (a * a) * d[1]
    ea = d[4] - d[2]
    t = d[3] - d[1]
    oa = a * t
    return {RP: e1 + o1, RM: e1 - o1, dp: ea + oa, dm: ea - oa,
            I: (d[5] - d[3]) - (a * a) * t, Z: (d[0] - d[2]) + (1.0 / (a * a)) * ea}


def _xf_s3(d):
    p, q = P_, Q_
    o1, o2 = d[3] - d[1], d[5] - d[3]
    e1, e2 = d[2] - d[0], d[4] - d[2]
    op_, oq_, or_ = o2 - (q * q) * o1, o2 - (p * p) * o1, (d[5] + d[1]) - S_ * d[3]
    ep_, eq_, er_ = p * e2 - q * e1, q * e2 - p * e1, (d[4] + d[0]) - S_ * d[2]
    return {PP: op_ + ep_, PM: op_ - ep_, QP: oq_ + eq_, QM: oq_ - eq_,
            RP: or_ + er_, RM: or_ - er_}


XF = {"S": _xf_s, "S1": lambda d: _xf_a1(d, Q_, QP, QM), "S2": lambda d: _xf_a1(d, P_, PP, PM),
      "S3": _xf_s3}

_AT = np.zeros((4, 8))
for _j, _a in {PP: P_, PM: -P_, QP: Q_, QM: -Q_, RP: 1.0, RM: -1.0}.items():
    _AT[:, _j] = [_a ** _i for _i in range(4)]
_AT[0, Z] = 1.0
_AT[3, I] = 1.0


def _solve_g(name):
    bt = XF[name]([np.eye(6)[k] for k in range(6)])
    dirs = sorted(bt)
    m = np.stack([np.concatenate([_AT[i, j] * bt[j] for i in range(4)]) for j in dirs], axis=1)
    sol = []
    for k in range(3):
        rhs = np.concatenate([np.eye(6)[i + k] for i in range(4)])
        s = np.linalg.lstsq(m, rhs, rcond=None)[0]
        assert np.allclose(m @ s, rhs, atol=1e-10)
        sol.append(s)
    sol = np.array(sol)
    sol[np.abs(sol) < 1e-12] = 0.0
    sol[np.abs(sol - 1) < 1e-12] = 1.0
    return {j: sol[:, n] for n, j in enumerate(dirs)}


GS = {n: _solve_g(n) for n in XF}


def _set_of(b, g):
    if g == 0:
        return "S1"
    if g == 1:
        return "S2"
    if g == 2 and b > 0:
        return "S3"
    return "S"


BLK = {j: [(b, g) for b in range(3) for g in range(6) if j in GS[_set_of(b, g)]] for j in range(8)}
OFF = {}
NBLK = 0
for _j in range(8):
    OFF[_j] = NBLK
    NBLK += 16 if len(BLK[_j]) > 8 else 8
POS = {(j, bg): OFF[j] + n for j in range(8) for n, bg in enumerate(BLK[j])}
VR = 8 * (NBLK + 6)

PEEL = (1, 1, 2, 3, 4)
QB = 5
LEAD_PEEL = (2, 3, 3, 3, 1, 1)
LEAD = 1
WAITS = (0, 1, 2, 4)
RG = 16
N0 = 24
FLUSH0 = 25
TAIL = (2, 1, 1)

NP = sum(PEEL)
NIT = (NQ - NP) // QB
assert NP + NIT * QB == NQ
SIZES = list(PEEL) + [QB] * NIT
STARTS = [sum(SIZES[:b]) for b in range(len(SIZES) + 1)]
QMAX = max(SIZES)


def _quad_of(n):
    if isinstance(n, int):
        m = n - N0
        return n if n < N0 else N0 + (m // 16) * 16 + (m % 4) * 4 + (m % 16) // 4
    m = jnp.maximum(n - N0, 0)
    return jnp.where(n < N0, n, N0 + (m // 16) * 16 + (m % 4) * 4 + (m % 16) // 4)


def _out_plan():
    plan = {FLUSH0 - 1: [(lambda ref, r=r: ref.at[pl.ds(0, N0 // 4), r]) for r in range(RG)]}
    for sq in range((NQ - N0) // 4):
        g0, j = N0 // 4 + 4 * (sq // 4), sq % 4
        b0 = 0
        for n in ((4,) if N0 + 4 * sq + 4 < NQ else TAIL):
            pos = N0 + 4 * sq + b0 + n - 1
            if pos == NQ - 1:
                break
            if n == 1:
                sls = [lambda ref, g=g0 + b0, j=j: ref.at[g, pl.ds(4 * j, 4)]]
            else:
                sls = [(lambda ref, g=g0 + b0, n=n, r=4 * j + k: ref.at[pl.ds(g, n), r])
                       for k in range(4)]
            plan.setdefault(pos, []).extend(sls)
            b0 += n
    out = {}
    for pos, sls in plan.items():
        i, t = divmod(pos - NP, QB)
        out.setdefault(((len(PEEL) + i) % 2, t), []).append((i, sls))
    return out


OUT_PLAN = _out_plan()

_need = [min(4 * max(_quad_of(n) for n in range(STARTS[b + 1])) + 4, H - 2)
         for b in range(len(SIZES))]
BOUNDS = [0] + _need[:len(PEEL) + 1]
LOOP_WAIT = {}
for _n, _i in enumerate(WAITS):
    _last = WAITS[_n + 1] - 1 if _n + 1 < len(WAITS) else NIT - 2
    LOOP_WAIT[_i] = len(BOUNDS) - 1
    BOUNDS.append(_need[len(PEEL) + 1 + _last])
assert BOUNDS[-1] == H - 2 and all(a < b for a, b in zip(BOUNDS, BOUNDS[1:]))
NCHUNK = len(BOUNDS) - 1


def _kernel(x_hbm, w_hbm, o_hbm, xbuf, obuf, wbuf, u_ref, v0_ref, v1_ref, sem_w, sem_in, sem_out):
    v_refs = (v0_ref, v1_ref)
    npeel = len(PEEL)

    def in_copy(c):
        rows = pl.ds(BOUNDS[c], BOUNDS[c + 1] - BOUNDS[c])
        return pltpu.make_async_copy(x_hbm.at[rows], xbuf.at[rows], sem_in.at[c])

    w_copy = pltpu.make_async_copy(w_hbm, wbuf, sem_w)
    halo_copy = pltpu.make_async_copy(x_hbm.at[pl.ds(H - 2, 2)], xbuf.at[pl.ds(H - 2, 2)],
                                      sem_in.at[0])
    w_copy.start()
    halo_copy.start(priority=1)
    for c in range(NCHUNK):
        in_copy(c).start(priority=1)

    def pack(v):
        return pltpu.bitcast(v.astype(bf16), u32)

    def unpack(u):
        return pltpu.bitcast(u, bf16)

    def prep_weights():
        eye = (jax.lax.broadcasted_iota(jnp.int32, (C, C), 0)
               == jax.lax.broadcasted_iota(jnp.int32, (C, C), 1)).astype(bf16)
        for j in range(8):
            pieces = []
            for (b, g) in BLK[j]:
                gc = GS[_set_of(b, g)][j]
                acc = None
                for k in range(3):
                    if gc[k] == 0.0:
                        continue
                    r0 = ((2 - k) * 3 + b) * C + 16 * g
                    t = wbuf[r0:r0 + 16, :].astype(f32)
                    t = t if gc[k] == 1.0 else float(gc[k]) * t
                    acc = t if acc is None else acc + t
                pieces.append(acc)
            ut = jnp.concatenate(pieces, axis=0).astype(bf16)
            u = jax.lax.dot_general(eye, ut, (((1,), (1,)), ((), ())),
                                    preferred_element_type=f32)
            u_ref[:, 16 * OFF[j]:16 * (OFF[j] + len(BLK[j]))] = pack(u)

    def stage_a(quads, slot, lead):
        v_ref = v_refs[slot]
        items = [(t, g) for t in range(len(quads)) for g in range(6)]
        wrapped = {}
        zeros = jnp.zeros((16, WP - W), bf16)

        def transform(t, g):
            def row(k):
                h = 4 * quads[t] - 2 + k
                return h % H if isinstance(h, int) else h
            d = [jnp.concatenate([xbuf[row(k), 16 * g:16 * g + 16, :], zeros], axis=1).astype(f32)
                 for k in range(6)]
            rows = {}
            for j, v in XF[_set_of(0, g)](d).items():
                rows[j] = t * VR + 8 * POS[(j, (0, g))]
                v_ref[rows[j]:rows[j] + 8, :] = pack(v)
            if _set_of(0, g) != _set_of(1, g):
                rows = {}
                for n, (j, v) in enumerate(XF[_set_of(1, g)](d).items()):
                    rows[j] = t * VR + 8 * (NBLK + n)
                    v_ref[rows[j]:rows[j] + 8, :] = pack(v)
            wrapped[(t, g)] = {}
            for j, r0 in rows.items():
                u = v_ref[r0:r0 + 8, :]
                wrapped[(t, g)][j] = jnp.concatenate([u[:, :W], u[:, 2 * W - WP:W]], axis=1)

        def shift(t, g):
            for j, u in wrapped.pop((t, g)).items():
                for b in (1, 2):
                    r0 = t * VR + 8 * POS[(j, (b, g))]
                    v_ref[r0:r0 + 8, :] = pltpu.roll(u, b, axis=1)

        for m in range(len(items) + lead):
            if m < len(items):
                transform(*items[m])
            if m >= lead:
                shift(*items[m - lead])

    def stage_b(quad, slot, t, after=None):
        v_ref = v_refs[slot]
        p, q = P_, Q_
        og, h0 = quad // 4, (quad % 4) * 4
        for (l0, l1) in ((0, 128), (128, W)):
            def mm(j):
                k0, k1 = OFF[j], OFF[j] + len(BLK[j])
                return jnp.dot(unpack(u_ref[:, 16 * k0:16 * k1]),
                               unpack(v_ref[t * VR + 8 * k0:t * VR + 8 * k1, l0:l1]),
                               preferred_element_type=f32)
            m1, m2 = mm(PP), mm(PM)
            s1, d1 = m1 + m2, m1 - m2
            m3, m4 = mm(QP), mm(QM)
            s2, d2 = m3 + m4, m3 - m4
            m5, m6 = mm(RP), mm(RM)
            s3, d3 = m5 + m6, m5 - m6
            obuf[og, h0 + 1, :, l0:l1] = ((p * d1 + q * d2) + d3).astype(bf16)
            obuf[og, h0 + 2, :, l0:l1] = (((p * p) * s1 + (q * q) * s2) + s3).astype(bf16)
            obuf[og, h0, :, l0:l1] = (((s1 + s2) + s3) + mm(Z)).astype(bf16)
            obuf[og, h0 + 3, :, l0:l1] = (
                (((p ** 3) * d1 + (q ** 3) * d2) + d3) + mm(I)).astype(bf16)
            if after is not None:
                after(l0, l1)

    def out_start(slicers):
        for sl in slicers:
            pltpu.make_async_copy(sl(obuf), sl(o_hbm), sem_out).start(priority=1)

    w_copy.wait()
    prep_weights()
    halo_copy.wait()
    in_copy(0).wait()
    stage_a(list(range(SIZES[0])), 0, LEAD_PEEL[0])
    for b in range(npeel):
        in_copy(b + 1).wait()
        for t in range(SIZES[b]):
            stage_b(STARTS[b] + t, b % 2, t)
        stage_a(list(range(STARTS[b + 1], STARTS[b + 2])), (b + 1) % 2, LEAD_PEEL[b + 1])

    def body(i, carry):
        for it, c in LOOP_WAIT.items():
            pl.when(i == it)(lambda c=c: in_copy(c).wait())
        n0 = NP + i * QB
        n1 = jnp.minimum(n0 + QB, NQ - QB)

        def last_rows(l0, l1):
            sl = lambda ref: ref.at[H // RG - 1, pl.ds(RG - 4, 4), :, pl.ds(l0, l1 - l0)]
            pl.when(i == NIT - 1)(functools.partial(out_start, [sl]))

        def half(s):
            for t in range(QB):
                is_last = t == QB - 1 and s == (npeel + NIT - 1) % 2
                stage_b(_quad_of(n0 + t), s, t, last_rows if is_last else None)
                for (it, sls) in OUT_PLAN.get((s, t), []):
                    pl.when(i == it)(functools.partial(out_start, sls))
            stage_a([_quad_of(n1 + t) for t in range(QB)], 1 - s, LEAD)

        pl.when((i + npeel) % 2 == 0)(functools.partial(half, 0))
        pl.when((i + npeel) % 2 == 1)(functools.partial(half, 1))
        return carry

    jax.lax.fori_loop(0, NIT, body, 0)
    pltpu.make_async_copy(obuf, o_hbm, sem_out).wait()


@jax.jit
def pallas_standalone__fft_conv__vision_kernel(
    x: jax.Array,
    w: jax.Array,
):
    xt = jnp.transpose(x[0], (0, 2, 1))
    w2 = w.reshape(9 * C, C)
    yt = pl.pallas_call(
        _kernel,
        in_specs=[pl.BlockSpec(memory_space=pl.ANY), pl.BlockSpec(memory_space=pl.ANY)],
        out_specs=pl.BlockSpec(memory_space=pl.ANY),
        out_shape=jax.ShapeDtypeStruct((H // RG, RG, C, W), bf16),
        scratch_shapes=[
            pltpu.VMEM((H, C, W), bf16),
            pltpu.VMEM((H // RG, RG, C, W), bf16),
            pltpu.VMEM((9 * C, C), bf16),
            pltpu.VMEM((C // 2, 16 * NBLK), u32),
            pltpu.VMEM((QMAX * VR, WP), u32),
            pltpu.VMEM((QMAX * VR, WP), u32),
            pltpu.SemaphoreType.DMA(()),
            pltpu.SemaphoreType.DMA((NCHUNK,)),
            pltpu.SemaphoreType.DMA(()),
        ],
        compiler_params=pltpu.CompilerParams(
            vmem_limit_bytes=64 * 1024 * 1024, disable_bounds_checks=True),
    )(xt, w2)
    return jnp.transpose(yt.reshape(H, C, W), (0, 2, 1))[None]
```

```python
import functools

import numpy as np
import jax
import jax.numpy as jnp
import jax.experimental.pallas as pl
import jax.experimental.pallas.tpu as pltpu

H = W = 224
C = 96
NQ = H // 4
WP = 256
bf16, f32, u32 = jnp.bfloat16, jnp.float32, jnp.uint32

P_ = 1.75
Q_ = 1.0 / P_
S_ = P_ * P_ + Q_ * Q_
Z, I, PP, PM, QP, QM, RP, RM = range(8)


def _xf_s(d):
    p, q = P_, Q_
    a2 = (p * p) * d[2]
    eq = d[4] - (q * q) * d[2]
    ep = d[4] - a2
    oq = p * d[3] - q * d[1]
    op = q * d[3] - p * d[1]
    return {Z: d[0] + eq - a2, PP: eq + oq, PM: eq - oq, QP: ep + op, QM: ep - op,
            I: (d[1] + d[5]) - S_ * d[3]}


def _xf_a1(d, a, dp, dm):
    e1 = d[4] - (a * a) * d[2]
    o1 = d[3] - (a * a) * d[1]
    ea = d[4] - d[2]
    t = d[3] - d[1]
    oa = a * t
    return {RP: e1 + o1, RM: e1 - o1, dp: ea + oa, dm: ea - oa,
            I: (d[5] - d[3]) - (a * a) * t, Z: (d[0] - d[2]) + (1.0 / (a * a)) * ea}


def _xf_s3(d):
    p, q = P_, Q_
    o1, o2 = d[3] - d[1], d[5] - d[3]
    e1, e2 = d[2] - d[0], d[4] - d[2]
    op_, oq_, or_ = o2 - (q * q) * o1, o2 - (p * p) * o1, (d[5] + d[1]) - S_ * d[3]
    ep_, eq_, er_ = p * e2 - q * e1, q * e2 - p * e1, (d[4] + d[0]) - S_ * d[2]
    return {PP: op_ + ep_, PM: op_ - ep_, QP: oq_ + eq_, QM: oq_ - eq_,
            RP: or_ + er_, RM: or_ - er_}


XF = {"S": _xf_s, "S1": lambda d: _xf_a1(d, Q_, QP, QM), "S2": lambda d: _xf_a1(d, P_, PP, PM),
      "S3": _xf_s3}

_AT = np.zeros((4, 8))
for _j, _a in {PP: P_, PM: -P_, QP: Q_, QM: -Q_, RP: 1.0, RM: -1.0}.items():
    _AT[:, _j] = [_a ** _i for _i in range(4)]
_AT[0, Z] = 1.0
_AT[3, I] = 1.0


def _solve_g(name):
    bt = XF[name]([np.eye(6)[k] for k in range(6)])
    dirs = sorted(bt)
    m = np.stack([np.concatenate([_AT[i, j] * bt[j] for i in range(4)]) for j in dirs], axis=1)
    sol = []
    for k in range(3):
        rhs = np.concatenate([np.eye(6)[i + k] for i in range(4)])
        s = np.linalg.lstsq(m, rhs, rcond=None)[0]
        assert np.allclose(m @ s, rhs, atol=1e-10)
        sol.append(s)
    sol = np.array(sol)
    sol[np.abs(sol) < 1e-12] = 0.0
    sol[np.abs(sol - 1) < 1e-12] = 1.0
    return {j: sol[:, n] for n, j in enumerate(dirs)}


GS = {n: _solve_g(n) for n in XF}


def _set_of(b, g):
    if g == 0:
        return "S1"
    if g == 1:
        return "S2"
    if g == 2 and b > 0:
        return "S3"
    return "S"


BLK = {j: [(b, g) for b in range(3) for g in range(6) if j in GS[_set_of(b, g)]] for j in range(8)}
OFF = {}
NBLK = 0
for _j in range(8):
    OFF[_j] = NBLK
    NBLK += 16 if len(BLK[_j]) > 8 else 8
POS = {(j, bg): OFF[j] + n for j in range(8) for n, bg in enumerate(BLK[j])}
VR = 8 * (NBLK + 6)

PEEL = (1, 1, 2, 3, 4)
QB = 5
LEAD_PEEL = (2, 3, 3, 3, 1, 1)
LEAD = 1
WAITS = (0, 1, 2, 4)
RG = 16
N0 = 24
FLUSH0 = 25
TAIL = (2, 1, 1)

NP = sum(PEEL)
NIT = (NQ - NP) // QB
assert NP + NIT * QB == NQ
SIZES = list(PEEL) + [QB] * NIT
STARTS = [sum(SIZES[:b]) for b in range(len(SIZES) + 1)]
QMAX = max(SIZES)


def _quad_of(n):
    static = isinstance(n, int)
    m = max(n - N0, 0) if static else jnp.maximum(n - N0, 0)
    banded = N0 + ((m >> 4) << 4) + ((m & 3) << 2) + ((m >> 2) & 3)
    return (n if n < N0 else banded) if static else jnp.where(n < N0, n, banded)


def _out_plan():
    first = [(lambda ref, r=r: ref.at[pl.ds(0, N0 // 4), r]) for r in range(RG)]
    plan = {FLUSH0 - 1: first[:RG // 2], FLUSH0 + 1: first[RG // 2:]}
    for sq in range((NQ - N0) // 4):
        g0, j = N0 // 4 + 4 * (sq // 4), sq % 4
        b0 = 0
        for n in ((4,) if N0 + 4 * sq + 4 < NQ else TAIL):
            pos = N0 + 4 * sq + b0 + n - 1
            if n == 1:
                sls = [lambda ref, g=g0 + b0, j=j: ref.at[g, pl.ds(4 * j, 4)]]
            else:
                sls = [(lambda ref, g=g0 + b0, n=n, r=4 * j + k: ref.at[pl.ds(g, n), r])
                       for k in range(4)]
            plan.setdefault(pos, []).extend(sls)
            b0 += n
    out = {}
    for pos, sls in plan.items():
        i, t = divmod(pos - NP, QB)
        out.setdefault(((len(PEEL) + i) % 2, t), []).append((i, sls))
    return out


OUT_PLAN = _out_plan()

_need = [min(4 * max(_quad_of(n) for n in range(STARTS[b + 1])) + 4, H - 2)
         for b in range(len(SIZES))]
BOUNDS = [0] + _need[:len(PEEL) + 1]
LOOP_WAIT = {}
for _n, _i in enumerate(WAITS):
    _last = WAITS[_n + 1] - 1 if _n + 1 < len(WAITS) else NIT - 2
    LOOP_WAIT[_i] = len(BOUNDS) - 1
    BOUNDS.append(_need[len(PEEL) + 1 + _last])
assert BOUNDS[-1] == H - 2 and all(a < b for a, b in zip(BOUNDS, BOUNDS[1:]))
NCHUNK = len(BOUNDS) - 1
NSEM = 4


def _kernel(x_hbm, w_hbm, o_hbm, xbuf, obuf, wbuf, u_ref, v0_ref, v1_ref, sem_in, sem_out):
    v_refs = (v0_ref, v1_ref)
    npeel = len(PEEL)

    def in_copy(c):
        rows = pl.ds(BOUNDS[c], BOUNDS[c + 1] - BOUNDS[c])
        return pltpu.make_async_copy(x_hbm.at[rows], xbuf.at[rows], sem_in.at[c % NSEM])

    def in_wait(c):
        in_copy(c).wait()
        if c + NSEM < NCHUNK:
            in_copy(c + NSEM).start(priority=1)

    w_copy = pltpu.make_async_copy(w_hbm, wbuf, sem_out)
    halo_copy = pltpu.make_async_copy(x_hbm.at[pl.ds(H - 2, 2)], xbuf.at[pl.ds(H - 2, 2)],
                                      sem_in.at[0])
    w_copy.start()
    halo_copy.start(priority=1)
    for c in range(NSEM):
        in_copy(c).start(priority=1)

    def pack(v):
        return pltpu.bitcast(v.astype(bf16), u32)

    def unpack(u):
        return pltpu.bitcast(u, bf16)

    def prep_weights():
        eye = (jax.lax.broadcasted_iota(jnp.int32, (C, C), 0)
               == jax.lax.broadcasted_iota(jnp.int32, (C, C), 1)).astype(bf16)
        for j in range(8):
            pieces = []
            for (b, g) in BLK[j]:
                gc = GS[_set_of(b, g)][j]
                acc = None
                for k in range(3):
                    if gc[k] == 0.0:
                        continue
                    r0 = ((2 - k) * 3 + b) * C + 16 * g
                    t = wbuf[r0:r0 + 16, :].astype(f32)
                    t = t if gc[k] == 1.0 else float(gc[k]) * t
                    acc = t if acc is None else acc + t
                pieces.append(acc)
            ut = jnp.concatenate(pieces, axis=0).astype(bf16)
            u = jax.lax.dot_general(eye, ut, (((1,), (1,)), ((), ())),
                                    preferred_element_type=f32)
            u_ref[:, 16 * OFF[j]:16 * (OFF[j] + len(BLK[j]))] = pack(u)

    def stage_a(quads, slot, lead):
        v_ref = v_refs[slot]
        items = [(t, g) for t in range(len(quads)) for g in range(6)]
        wrapped = {}
        zeros = jnp.zeros((16, WP - W), bf16)

        def transform(t, g):
            def row(k):
                h = 4 * quads[t] - 2 + k
                return h % H if isinstance(h, int) else h
            d = [jnp.concatenate([xbuf[row(k), 16 * g:16 * g + 16, :], zeros], axis=1).astype(f32)
                 for k in range(6)]
            rows = {}
            for j, v in XF[_set_of(0, g)](d).items():
                rows[j] = t * VR + 8 * POS[(j, (0, g))]
                v_ref[rows[j]:rows[j] + 8, :] = pack(v)
            if _set_of(0, g) != _set_of(1, g):
                rows = {}
                for n, (j, v) in enumerate(XF[_set_of(1, g)](d).items()):
                    rows[j] = t * VR + 8 * (NBLK + n)
                    v_ref[rows[j]:rows[j] + 8, :] = pack(v)
            wrapped[(t, g)] = {}
            for j, r0 in rows.items():
                u = v_ref[r0:r0 + 8, :]
                wrapped[(t, g)][j] = jnp.concatenate([u[:, :W], u[:, 2 * W - WP:W]], axis=1)

        def shift(t, g):
            for j, u in wrapped.pop((t, g)).items():
                for b in (1, 2):
                    r0 = t * VR + 8 * POS[(j, (b, g))]
                    v_ref[r0:r0 + 8, :] = pltpu.roll(u, b, axis=1)

        for m in range(len(items) + lead):
            if m < len(items):
                transform(*items[m])
            if m >= lead:
                shift(*items[m - lead])

    def stage_b(quad, slot, t):
        v_ref = v_refs[slot]
        p, q = P_, Q_
        og, h0 = quad >> 2, (quad & 3) << 2
        for (l0, l1) in ((0, 128), (128, W)):
            def mm(j):
                k0, k1 = OFF[j], OFF[j] + len(BLK[j])
                return jnp.dot(unpack(u_ref[:, 16 * k0:16 * k1]),
                               unpack(v_ref[t * VR + 8 * k0:t * VR + 8 * k1, l0:l1]),
                               preferred_element_type=f32)
            m1, m2 = mm(PP), mm(PM)
            s1, d1 = m1 + m2, m1 - m2
            m3, m4 = mm(QP), mm(QM)
            s2, d2 = m3 + m4, m3 - m4
            m5, m6 = mm(RP), mm(RM)
            s3, d3 = m5 + m6, m5 - m6
            obuf[og, h0 + 1, :, l0:l1] = ((p * d1 + q * d2) + d3).astype(bf16)
            obuf[og, h0 + 2, :, l0:l1] = (((p * p) * s1 + (q * q) * s2) + s3).astype(bf16)
            obuf[og, h0, :, l0:l1] = (((s1 + s2) + s3) + mm(Z)).astype(bf16)
            obuf[og, h0 + 3, :, l0:l1] = (
                (((p ** 3) * d1 + (q ** 3) * d2) + d3) + mm(I)).astype(bf16)

    def out_start(slicers):
        for sl in slicers:
            pltpu.make_async_copy(sl(obuf), sl(o_hbm), sem_out).start(priority=1)

    w_copy.wait()
    prep_weights()
    halo_copy.wait()
    in_wait(0)
    stage_a(list(range(SIZES[0])), 0, LEAD_PEEL[0])
    for b in range(npeel):
        in_wait(b + 1)
        for t in range(SIZES[b]):
            stage_b(STARTS[b] + t, b % 2, t)
        stage_a(list(range(STARTS[b + 1], STARTS[b + 2])), (b + 1) % 2, LEAD_PEEL[b + 1])

    def half(k, odd):
        for it, c in LOOP_WAIT.items():
            if it % 2 == odd:
                pl.when(k == it // 2)(functools.partial(in_wait, c))
        s = (npeel + odd) % 2
        n0 = NP + odd * QB + k * (2 * QB)
        n1 = jnp.minimum(n0 + QB, NQ - QB)
        for t in range(QB):
            stage_b(_quad_of(n0 + t), s, t)
            for (it, sls) in OUT_PLAN.get((s, t), []):
                pl.when(k == it // 2)(functools.partial(out_start, sls))
        stage_a([_quad_of(n1 + t) for t in range(QB)], 1 - s, LEAD)

    def body(k, carry):
        half(k, 0)
        pl.when(2 * k + 1 < NIT)(functools.partial(half, k, 1))
        return carry

    jax.lax.fori_loop(0, (NIT + 1) // 2, body, 0)
    pltpu.make_async_copy(obuf, o_hbm, sem_out).wait()


@jax.jit
def pallas_standalone__fft_conv__vision_kernel(
    x: jax.Array,
    w: jax.Array,
):
    xt = jnp.transpose(x[0], (0, 2, 1))
    w2 = w.reshape(9 * C, C)
    yt = pl.pallas_call(
        _kernel,
        in_specs=[pl.BlockSpec(memory_space=pl.ANY), pl.BlockSpec(memory_space=pl.ANY)],
        out_specs=pl.BlockSpec(memory_space=pl.ANY),
        out_shape=jax.ShapeDtypeStruct((H // RG, RG, C, W), bf16),
        scratch_shapes=[
            pltpu.VMEM((H, C, W), bf16),
            pltpu.VMEM((H // RG, RG, C, W), bf16),
            pltpu.VMEM((9 * C, C), bf16),
            pltpu.VMEM((C // 2, 16 * NBLK), u32),
            pltpu.VMEM((QMAX * VR, WP), u32),
            pltpu.VMEM((QMAX * VR, WP), u32),
            pltpu.SemaphoreType.DMA((NSEM,)),
            pltpu.SemaphoreType.DMA(()),
        ],
        compiler_params=pltpu.CompilerParams(
            vmem_limit_bytes=64 * 1024 * 1024, disable_bounds_checks=True),
    )(xt, w2)
    return jnp.transpose(yt.reshape(H, C, W), (0, 2, 1))[None]
```
